```python
import jax
import jax.numpy as jnp

def _softmax(x, axis=-1):
    return jax.nn.softmax(x, axis=axis)
def _gelu(x):
    return jax.nn.gelu(x, approximate=True)
def _silu(x):
    return jax.nn.silu(x)
def _sigmoid(x):
    return jax.nn.sigmoid(x)
def _layernorm(x, axis=-1, eps=1e-5):
    m = jnp.mean(x, axis=axis, keepdims=True)
    v = jnp.var(x, axis=axis, keepdims=True)
    return (x - m) / jnp.sqrt(v + eps)
def _scatter_add(tgt, idx, src, axis=0):
    return tgt.at[idx].add(src)
def _segment_sum(src, seg, n):
    return jax.ops.segment_sum(src, seg, n)
class _Rng:
    def __init__(self, key):
        self._k = key
    def _next(self):
        self._k, sub = jax.random.split(self._k)
        return sub
    def normal(self, shape):
        return jax.random.normal(self._next(), shape, dtype=jnp.bfloat16)
    def randint(self, lo, hi, shape):
        return jax.random.randint(self._next(), shape, lo, hi, dtype=jnp.int32)
    def uniform(self, shape, lo=0.0, hi=1.0):
        return jax.random.uniform(self._next(), shape, jnp.bfloat16, lo, hi)
    def permutation(self, n):
        return jax.random.permutation(self._next(), n)


kernel_name = 'standalone__depthwise_separable__vision'

def setup_inputs():
    _rng = _Rng(jax.random.key(int.from_bytes(__import__("os").urandom(4), "little")))
    _w = (lambda a: (lambda t: t.astype(jnp.bfloat16) if jnp.issubdtype(t.dtype, jnp.floating) else t)(jnp.asarray(a)))
    H = W = 384
    C = 384
    k = 1
    return {
        "x": _w((lambda *s: _rng.normal(s) * 0.05)(1, H, W, C)),
        "dw": _w((lambda *s: _rng.normal(s) * 0.05)(k, k, C)),
        "pw": _w((lambda *s: _rng.normal(s) * 0.05)(C, C)),
    }

def reference(x, dw, pw):
    B, H, W, C = x.shape
    k = dw.shape[0]
    pad = k // 2
    xp = jnp.pad(x, ((0,0),(pad,pad),(pad,pad),(0,0)))
    out = jnp.zeros_like(x)
    for i in range(k):
        for j in range(k):
            out = out + xp[:, i:i+H, j:j+W, :] * dw[i, j][None, None, None, :]
    return jnp.einsum('bhwc,cd->bhwd', out, pw)
```

```python
import jax
import jax.numpy as jnp
import jax.experimental.pallas as pl
import jax.experimental.pallas.tpu as pltpu

S = 6
T = 384
TW = 48
K1 = 32
TAIL = 48
BURST = 16


def _kernel(x_hbm, dw_hbm, pw_hbm, o_hbm, buf, dw_v, pw_v, w_v, rsem, wsem, psem):
    _, P, C = buf.shape
    n = P // T
    wpc = T // TW

    def rows(start, size):
        return (slice(None), pl.ds(start, size))

    def rd(start, size, sem):
        sl = rows(start, size)
        return pltpu.make_async_copy(x_hbm.at[sl], buf.at[sl], sem)

    def wr(j):
        sl = rows(pl.multiple_of(j * TW, 8), TW)
        return pltpu.make_async_copy(buf.at[sl], o_hbm.at[sl], wsem.at[0])

    cp_dw = pltpu.make_async_copy(dw_hbm, dw_v, psem.at[0])
    cp_pw = pltpu.make_async_copy(pw_hbm, pw_v, psem.at[1])
    cp_dw.start()
    cp_pw.start()

    def issue_rd(k, c):
        rd(pl.multiple_of(k * T, T), T, rsem.at[k]).start()
        return c

    jax.lax.fori_loop(0, K1, issue_rd, 0)
    rd_rest = rd(K1 * T, P - K1 * T - TAIL, rsem.at[K1])
    rd_rest.start()
    rd_tail = rd(P - TAIL, TAIL, rsem.at[K1 + 1])
    rd_tail.start()

    cp_dw.wait()
    cp_pw.wait()
    dw_col = jnp.broadcast_to(dw_v[0].astype(jnp.float32), (C, C)).T
    w_v[...] = (dw_col * pw_v[...].astype(jnp.float32)).astype(w_v.dtype)

    def compute(k):
        r = pl.ds(pl.multiple_of(k * T, T), T)
        for s in range(S):
            buf[s, r, :] = jnp.dot(
                buf[s, r, :], w_v[...], preferred_element_type=jnp.float32
            ).astype(buf.dtype)

    def phase1(k, c):
        rd(pl.multiple_of(k * T, T), T, rsem.at[k]).wait()
        compute(k)
        return c

    jax.lax.fori_loop(0, K1, phase1, 0)
    rd_rest.wait()

    def issue_wr(j, c):
        wr(j).start()
        return c

    jax.lax.fori_loop(0, BURST, issue_wr, 0)
    rd_tail.wait()

    def phase2(k, nxt):
        compute(k)
        lim = jnp.minimum(nxt + BURST, (k + 1) * wpc)
        jax.lax.fori_loop(nxt, lim, issue_wr, 0)
        return lim

    nxt = jax.lax.fori_loop(K1, n, phase2, BURST)
    jax.lax.fori_loop(nxt, n * wpc, issue_wr, 0)
    pltpu.make_async_copy(buf, o_hbm, wsem.at[0]).wait()


@jax.jit
def pallas_standalone__depthwise_separable__vision_kernel(
    x: jax.Array,
    dw: jax.Array,
    pw: jax.Array,
):
    B, H, W, C = x.shape
    assert dw.shape == (1, 1, C) and pw.shape == (C, C)
    P = (B * H * W) // S
    assert P * S == B * H * W and P % T == 0

    out = pl.pallas_call(
        _kernel,
        in_specs=[pl.BlockSpec(memory_space=pl.ANY)] * 3,
        out_specs=pl.BlockSpec(memory_space=pl.ANY),
        out_shape=jax.ShapeDtypeStruct((S, P, C), x.dtype),
        scratch_shapes=[
            pltpu.VMEM((S, P, C), x.dtype),
            pltpu.VMEM(dw.shape, dw.dtype),
            pltpu.VMEM(pw.shape, pw.dtype),
            pltpu.VMEM(pw.shape, x.dtype),
            pltpu.SemaphoreType.DMA((K1 + 2,)),
            pltpu.SemaphoreType.DMA((1,)),
            pltpu.SemaphoreType.DMA((2,)),
        ],
        compiler_params=pltpu.CompilerParams(vmem_limit_bytes=124 * 1024 * 1024),
    )(x.reshape(S, P, C), dw, pw)
    return out.reshape(B, H, W, C)
```

```python
import jax
import jax.numpy as jnp
import jax.experimental.pallas as pl
import jax.experimental.pallas.tpu as pltpu

S = 6
D = 2048
T = 512
WPAT = (48,) * 10 + (32,)
TR = 32
PPP = 20
TAILP = 3
THIN = (80, 88, 88, 80, 88, 88)
B0 = 3
FIRST = 5

Q = D // T
H = D // 2
PPG = D // TR
WSEM, TSEM = 2, 3
assert sum(WPAT) == T and sum(THIN) == T
assert Q & (Q - 1) == 0 and PPG & (PPG - 1) == 0


def _log2(v):
    return v.bit_length() - 1


def _kernel(x_hbm, dw_hbm, pw_hbm, o_hbm, buf, dw_v, pw_v, w_v, sem):
    NB, _, C = buf.shape
    nchunk = (NB // S) * Q
    npiece = (NB // S) * PPG
    nper = (npiece - TAILP - 1) // PPP
    restp = npiece - nper * PPP - TAILP
    assert B0 + len(THIN) * S <= nper + 1

    def rd(p, s):
        row = (p & (PPG - 1)) * TR
        if not isinstance(p, int):
            row = pl.multiple_of(row, TR)
        sl = (pl.ds((p >> _log2(PPG)) * S, S), pl.ds(row, TR))
        return pltpu.make_async_copy(x_hbm.at[sl], buf.at[sl], sem.at[s])

    def wr(sl):
        pltpu.make_async_copy(buf.at[sl], o_hbm.at[sl], sem.at[WSEM]).start()

    def write_chunk(c):
        blk = (c >> _log2(Q)) * S
        row = (c & (Q - 1)) * T
        for size in WPAT:
            r = row if isinstance(row, int) else pl.multiple_of(row, 16)
            wr((pl.ds(blk, S), pl.ds(r, size)))
            row = row + size

    cp_dw = pltpu.make_async_copy(dw_hbm, dw_v, sem.at[TSEM])
    cp_pw = pltpu.make_async_copy(pw_hbm, pw_v, sem.at[TSEM])
    cp_dw.start()
    cp_pw.start()
    for p in range(2 * PPP):
        rd(p, p // PPP).start()

    cp_dw.wait()
    cp_pw.wait()
    dw_col = jnp.broadcast_to(dw_v[0].astype(jnp.float32), (C, C)).T
    w_v[...] = (dw_col * pw_v[...].astype(jnp.float32)).astype(w_v.dtype)

    for p in range(PPP):
        rd(p, 0).wait()
    for p in range(PPP):
        rd(2 * PPP + p, 0).start()

    def step(k, carry):
        base, j, h = carry

        @pl.when(k <= nper)
        def _():
            for i in range(PPP):
                rd((k - 1) * PPP + i, (k - 1) & 1).wait()

        row = 0
        for n, size in enumerate(THIN):
            blk = k - (B0 + n * S)

            @pl.when((blk >= 0) & (blk < S))
            def _():
                wr((blk, pl.ds(row, size)))

            row += size

        @pl.when(k + 1 < nper)
        def _():
            for i in range(PPP):
                rd((k + 1) * PPP + i, (k + 1) & 1).start()

        @pl.when(k + 1 == nper)
        def _():
            for i in range(restp):
                rd(nper * PPP + i, nper % 2).start()
            for i in range(TAILP):
                rd(npiece - TAILP + i, TSEM).start()

        @pl.when(k == nper)
        def _():
            for i in range(restp):
                rd(nper * PPP + i, nper % 2).wait()
            for c in range(1, FIRST + 1):
                write_chunk(c)
            for i in range(TAILP):
                rd(npiece - TAILP + i, TSEM).wait()

        r = pl.ds(pl.multiple_of(h * H, H), H)
        for i in range(2):
            b = base + j + i
            buf[b, r, :] = jnp.dot(
                buf[b, r, :], w_v[...], preferred_element_type=jnp.float32
            ).astype(buf.dtype)

        @pl.when(k >= nper)
        def _():
            write_chunk(FIRST + 1 + k - nper)

        wrap = j == S - 2
        return (
            jnp.where(wrap & (h == 1), base + S, base),
            jnp.where(wrap, 0, j + 2),
            jnp.where(wrap, 1 - h, h),
        )

    zero = jnp.int32(0)
    jax.lax.fori_loop(2, NB + 2, step, (zero, zero, zero))

    def flush(c, carry):
        write_chunk(c)
        return carry

    jax.lax.fori_loop(FIRST + 3 + NB - nper, nchunk, flush, 0)
    pltpu.make_async_copy(buf, o_hbm, sem.at[WSEM]).wait()


@jax.jit
def pallas_standalone__depthwise_separable__vision_kernel(
    x: jax.Array,
    dw: jax.Array,
    pw: jax.Array,
):
    B, Hh, Ww, C = x.shape
    assert dw.shape == (1, 1, C) and pw.shape == (C, C)
    NB = (B * Hh * Ww) // D
    assert NB * D == B * Hh * Ww and NB % S == 0

    out = pl.pallas_call(
        _kernel,
        in_specs=[pl.BlockSpec(memory_space=pl.ANY)] * 3,
        out_specs=pl.BlockSpec(memory_space=pl.ANY),
        out_shape=jax.ShapeDtypeStruct((NB, D, C), x.dtype),
        scratch_shapes=[
            pltpu.VMEM((NB, D, C), x.dtype),
            pltpu.VMEM(dw.shape, dw.dtype),
            pltpu.VMEM(pw.shape, pw.dtype),
            pltpu.VMEM(pw.shape, x.dtype),
            pltpu.SemaphoreType.DMA((4,)),
        ],
        compiler_params=pltpu.CompilerParams(vmem_limit_bytes=112 * 1024 * 1024),
    )(x.reshape(NB, D, C), dw, pw)
    return out.reshape(B, Hh, Ww, C)
```

```python
import jax
import jax.numpy as jnp
import jax.experimental.pallas as pl
import jax.experimental.pallas.tpu as pltpu

D = 2048
SB = 12
TR = 32
U = 128
TS = 64
X = 16
G0 = 4
GS = 6
KH = 54
TAIL = 48
S = 6
T = 512
WPAT = (48,) * 10 + (32,)
FIRST = 5

SPD = D // TR
UPD = D // U
assert SPD == 64 and UPD == 16 and D // T == 4 and SB == 2 * S
assert sum(WPAT) == T and U // TS == TR // X and G0 * TR >= U
WSEM = (KH + 1) % 2
HSEM = 2


def _kernel(x_hbm, dw_hbm, pw_hbm, o_hbm, buf, hbuf, dw_v, pw_v, w_v, sem):
    NBB, _, C = buf.shape
    nslab = NBB // SB * SPD
    nunit = NBB // SB * UPD
    nchunk = NBB // S * (D // T)
    nchunk_h = SB // S * (D // T)
    KD = 1 + (nslab - G0) // GS
    assert KD <= KH

    def slab(p, s):
        row = (p & (SPD - 1)) * TR
        if not isinstance(p, int):
            row = pl.multiple_of(row, TR)
        sl = (pl.ds((p >> 6) * SB, SB), pl.ds(row, TR))
        return pltpu.make_async_copy(x_hbm.at[sl], buf.at[sl], sem.at[s])

    def rows_h(row, n, s):
        return pltpu.make_async_copy(
            x_hbm.at[pl.ds(NBB, SB), pl.ds(row, n)],
            hbuf.at[pl.ds(0, SB), pl.ds(row, n)],
            sem.at[s],
        )

    def last_group(g):
        end = nslab + SPD - KH if g == KH else G0 + g * GS
        copies = []
        for p in range(G0 + (g - 1) * GS, end):
            if p < nslab:
                copies.append(slab(p, g % 2))
            else:
                row = (KH + p - nslab) * TR
                n = min(TR, D - TAIL - row)
                if n > 0:
                    copies.append(rows_h(row, n, g % 2))
        return copies

    def tail():
        return [rows_h(r, 16, HSEM) for r in range(D - TAIL, D, 16)]

    def write_chunk(src, off, c):
        blk = (c >> 3) * SB + (c & 1) * S
        row = ((c >> 1) & 3) * T
        for size in WPAT:
            r = row if isinstance(row, int) else pl.multiple_of(row, 16)
            pltpu.make_async_copy(
                src.at[pl.ds(blk, S), pl.ds(r, size)],
                o_hbm.at[pl.ds(off + blk, S), pl.ds(r, size)],
                sem.at[WSEM],
            ).start()
            row = row + size

    def unit(ref, u):
        row = pl.multiple_of((u & (UPD - 1)) * U, U)
        return ref.at[pl.ds((u >> 4) * SB, SB), pl.ds(row, U)]

    def matmul(a, w):
        return jnp.dot(a, w, preferred_element_type=jnp.float32).astype(buf.dtype)

    cp_dw = pltpu.make_async_copy(dw_hbm, dw_v, sem.at[HSEM])
    cp_pw = pltpu.make_async_copy(pw_hbm, pw_v, sem.at[HSEM])
    cp_dw.start()
    cp_pw.start()
    for p in range(G0 + GS):
        slab(p, int(p >= G0)).start(priority=1)

    cp_dw.wait()
    cp_pw.wait()
    dw_col = jnp.broadcast_to(dw_v[0].astype(jnp.float32), (C, C)).T
    w = (dw_col * pw_v[...].astype(jnp.float32)).astype(w_v.dtype)
    w_v[...] = w
    hbuf[SB, pl.ds(0, C), :] = w

    for p in range(G0):
        slab(p, 0).wait()

    def read_step(k, carry):
        @pl.when((k >= 2) & (k <= KD))
        def _():
            for i in range(GS):
                slab(G0 + (k - 2) * GS + i, (k - 1) & 1).wait()

        for g in range(KD, KH):
            @pl.when(k == g + 1)
            def _():
                for c in last_group(g):
                    c.wait()

        @pl.when(k + 1 < KD)
        def _():
            for i in range(GS):
                slab(G0 + k * GS + i, (k + 1) & 1).start(priority=1)

        for g in range(KD, KH + 1):
            @pl.when(k + 1 == g)
            def _():
                for c in last_group(g) + (tail() if g == KH else []):
                    c.start(priority=1)

        v = unit(buf, k - 1)
        hrows = pl.ds(pl.multiple_of((k - 1) * TR, TR), TR)
        hsrc = x_hbm.at[pl.ds(NBB, SB), hrows]
        hdst = hbuf.at[pl.ds(0, SB), hrows]
        for b in range(SB):
            for s in range(U // TS):
                pltpu.make_async_copy(
                    hsrc.at[b, pl.ds(s * X, X)],
                    hdst.at[b, pl.ds(s * X, X)],
                    sem.at[HSEM],
                ).start()
                r = pl.ds(s * TS, TS)
                v[b, r, :] = matmul(v[b, r, :], hbuf[SB, pl.ds(0, C), :])
        return carry

    jax.lax.fori_loop(1, KH + 1, read_step, 0)

    for c in last_group(KH):
        c.wait()
    for c in range(FIRST):
        write_chunk(buf, 0, c)
    for c in tail():
        c.wait()
    rows_h(0, KH * TR, HSEM).wait()

    def buf_step(u, carry):
        v = unit(buf, u)
        for b in range(SB):
            v[b] = matmul(v[b], w_v[...])
        write_chunk(buf, 0, FIRST + u - KH)
        return carry

    jax.lax.fori_loop(KH, nunit, buf_step, 0)

    nxt = FIRST + nunit - KH
    left = nchunk - nxt
    assert all(FIRST + u - KH < (u + 1) // 4 * 2 for u in range(KH, nunit))
    assert all(j - left < (j + 1) // 4 * 2 for j in range(left, UPD))

    def hbuf_step(j, carry):
        v = unit(hbuf, j)
        for b in range(SB):
            v[b] = matmul(v[b], w_v[...])

        @pl.when(j < left)
        def _():
            write_chunk(buf, 0, nxt + j)

        @pl.when(j >= left)
        def _():
            write_chunk(hbuf, NBB, j - left)

        return carry

    jax.lax.fori_loop(0, UPD, hbuf_step, 0)
    for c in range(UPD - left, nchunk_h):
        write_chunk(hbuf, NBB, c)

    pltpu.make_async_copy(buf, o_hbm.at[pl.ds(0, NBB)], sem.at[WSEM]).wait()
    pltpu.make_async_copy(
        hbuf.at[pl.ds(0, SB)], o_hbm.at[pl.ds(NBB, SB)], sem.at[WSEM]
    ).wait()


@jax.jit
def pallas_standalone__depthwise_separable__vision_kernel(
    x: jax.Array,
    dw: jax.Array,
    pw: jax.Array,
):
    B, Hh, Ww, C = x.shape
    assert dw.shape == (1, 1, C) and pw.shape == (C, C)
    NB = (B * Hh * Ww) // D
    assert NB * D == B * Hh * Ww and NB % SB == 0

    out = pl.pallas_call(
        _kernel,
        in_specs=[pl.BlockSpec(memory_space=pl.ANY)] * 3,
        out_specs=pl.BlockSpec(memory_space=pl.ANY),
        out_shape=jax.ShapeDtypeStruct((NB, D, C), x.dtype),
        scratch_shapes=[
            pltpu.VMEM((NB - SB, D, C), x.dtype),
            pltpu.VMEM((SB + 1, D, C), x.dtype),
            pltpu.VMEM(dw.shape, dw.dtype),
            pltpu.VMEM(pw.shape, pw.dtype),
            pltpu.VMEM(pw.shape, x.dtype),
            pltpu.SemaphoreType.DMA((3,)),
        ],
        compiler_params=pltpu.CompilerParams(
            vmem_limit_bytes=114 * 1024 * 1024,
            disable_bounds_checks=True,
        ),
    )(x.reshape(NB, D, C), dw, pw)
    return out.reshape(B, Hh, Ww, C)
```

```python
import jax
import jax.numpy as jnp
import jax.experimental.pallas as pl
import jax.experimental.pallas.tpu as pltpu

D = 2048
SB = 12
TR = 16
G0 = 8
GS = 14
KH = 47
U = 128
TS = 64
X = 8
HR = 2 * X * (U // TS)
NSPLIT = 256
SPIN = 6
TAIL = 48
S = 6
T = 512
WPAT = (40, 40, 48) * 4
FIRST = 5

PPD = D // TR
UPD = D // U
HI = (KH + 1) * HR
assert PPD == 128 and UPD == 16 and D // T == 4 and SB == 2 * S
assert sum(WPAT) == T and G0 * TR >= U and GS * TR >= U
assert HR == 32 and (D - TAIL - HI) % TR == 0
WSEM = (KH + 1) % 2
HSEM = 2


def _kernel(x_hbm, dw_hbm, pw_hbm, o_hbm, buf, hbuf, dw_v, pw_v, w_v, cnt, sem):
    NBB, _, C = buf.shape
    npiece = NBB // SB * PPD
    nunit = NBB // SB * UPD
    nchunk = NBB // S * (D // T)
    nchunk_h = SB // S * (D // T)
    nbulk = npiece + (D - TAIL - HI) // TR
    KD = min(KH, 1 + (npiece - G0) // GS)

    def piece(p, s):
        row = (p & (PPD - 1)) * TR
        if not isinstance(p, int):
            row = pl.multiple_of(row, TR)
        sl = (pl.ds((p >> 7) * SB, SB), pl.ds(row, TR))
        return pltpu.make_async_copy(x_hbm.at[sl], buf.at[sl], sem.at[s])

    def rows_h(row, n, s):
        return pltpu.make_async_copy(
            x_hbm.at[pl.ds(NBB, SB), pl.ds(row, n)],
            hbuf.at[pl.ds(0, SB), pl.ds(row, n)],
            sem.at[s],
        )

    def bulk(lo, hi, s):
        return [
            piece(p, s) if p < npiece else rows_h(HI + (p - npiece) * TR, TR, s)
            for p in range(lo, hi)
        ]

    def group(g):
        return bulk(G0 + (g - 1) * GS, G0 + g * GS, g % 2)

    def rest():
        return bulk(G0 + KH * GS, nbulk, KH % 2)

    def tail():
        return [rows_h(r, 16, HSEM) for r in range(D - TAIL, D, 16)]

    def write_chunk(src, off, c):
        blk = (c >> 3) * SB + (c & 1) * S
        row = ((c >> 1) & 3) * T
        for size in WPAT:
            r = row if isinstance(row, int) else pl.multiple_of(row, 8)
            pltpu.make_async_copy(
                src.at[pl.ds(blk, S), pl.ds(r, size)],
                o_hbm.at[pl.ds(off + blk, S), pl.ds(r, size)],
                sem.at[WSEM],
            ).start()
            row = row + size

    def unit(ref, u):
        row = pl.multiple_of((u & (UPD - 1)) * U, U)
        return ref.at[pl.ds((u >> 4) * SB, SB), pl.ds(row, U)]

    def matmul(a, w):
        return jnp.dot(a, w, preferred_element_type=jnp.float32).astype(buf.dtype)

    cp_dw = pltpu.make_async_copy(dw_hbm, dw_v, sem.at[HSEM])
    cp_pw = pltpu.make_async_copy(pw_hbm, pw_v, sem.at[HSEM])
    cp_dw.start()
    cp_pw.start()
    for c in bulk(0, G0, 0) + group(1):
        c.start(priority=1)
    cnt[0] = 0

    cp_dw.wait()
    cp_pw.wait()
    dw_col = jnp.broadcast_to(dw_v[0].astype(jnp.float32), (C, C)).T
    w = (dw_col * pw_v[...].astype(jnp.float32)).astype(w_v.dtype)
    w_v[...] = w
    hbuf[SB, pl.ds(0, C), :] = w

    def paced_read(i, carry):
        r = pl.ds(pl.multiple_of((i & 1) * (HR // 2), HR // 2), HR // 2)
        pltpu.make_async_copy(
            x_hbm.at[NBB + (i >> 1), r], hbuf.at[i >> 1, r], sem.at[HSEM]
        ).start()

        def spin(_, c):
            cnt[0] = cnt[0] + 1
            return c

        return jax.lax.fori_loop(0, SPIN, spin, carry)

    jax.lax.fori_loop(0, 2 * SB, paced_read, 0)
    for c in bulk(0, G0, 0):
        c.wait()

    def read_step(k, carry):
        @pl.when((k >= 2) & (k <= KD))
        def _():
            for i in range(GS):
                piece(G0 + (k - 2) * GS + i, (k - 1) & 1).wait()

        for g in range(KD, KH):
            @pl.when(k == g + 1)
            def _():
                for c in group(g):
                    c.wait()

        @pl.when(k + 1 < KD)
        def _():
            for i in range(GS):
                piece(G0 + k * GS + i, (k + 1) & 1).start(priority=1)

        for g in range(KD, KH + 1):
            @pl.when(k + 1 == g)
            def _():
                for c in group(g):
                    c.start(priority=1)

        @pl.when(k == KH)
        def _():
            for c in rest() + tail():
                c.start(priority=1)

        v = unit(buf, k - 1)
        hrows = pl.ds(pl.multiple_of(k * HR, HR), HR)
        hsrc = x_hbm.at[pl.ds(NBB, SB), hrows]
        hdst = hbuf.at[pl.ds(0, SB), hrows]

        def small_read(b, row):
            pltpu.make_async_copy(
                hsrc.at[b, pl.ds(row, X)], hdst.at[b, pl.ds(row, X)], sem.at[HSEM]
            ).start()

        lo, hi = pl.ds(0, NSPLIT), pl.ds(NSPLIT, C - NSPLIT)
        for b in range(SB):
            for s in range(U // TS):
                r = pl.ds(s * TS, TS)
                a = v[b, r, :]
                small_read(b, 2 * s * X)
                y_lo = matmul(a, hbuf[SB, pl.ds(0, C), lo])
                small_read(b, (2 * s + 1) * X)
                y_hi = matmul(a, hbuf[SB, pl.ds(0, C), hi])
                v[b, r, lo] = y_lo
                v[b, r, hi] = y_hi
        return carry

    jax.lax.fori_loop(1, KH + 1, read_step, 0)

    for c in group(KH) + rest():
        c.wait()
    for c in range(FIRST):
        write_chunk(buf, 0, c)
    for c in tail():
        c.wait()
    rows_h(0, HI, HSEM).wait()

    def unit_matmul(ref, u):
        v = unit(ref, u)
        for b in range(SB):
            v[b] = matmul(v[b], w_v[...])

    def buf_step(m, carry):
        unit_matmul(buf, KH + m)

        @pl.when((m & 7) != 7)
        def _():
            write_chunk(buf, 0, FIRST + m - (m >> 3))

        return carry

    nb = nunit - KH
    assert all(FIRST + m - (m >> 3) < (KH + m + 1) // 4 * 2 for m in range(nb))
    jax.lax.fori_loop(0, nb, buf_step, 0)

    def hbuf_step(j, c):
        unit_matmul(hbuf, j)
        ready = c - nchunk < ((j + 1) >> 2) * 2

        @pl.when(c < nchunk)
        def _():
            write_chunk(buf, 0, c)

        @pl.when((c >= nchunk) & ready)
        def _():
            write_chunk(hbuf, NBB, c - nchunk)

        return jnp.where(ready, c + 1, c)

    nxt = FIRST + nb - (nb >> 3)
    jax.lax.fori_loop(0, UPD, hbuf_step, jnp.int32(nxt))
    for j in range(UPD):
        nxt += nxt - nchunk < (j + 1) // 4 * 2
    assert nxt >= nchunk
    for c in range(nxt - nchunk, nchunk_h):
        write_chunk(hbuf, NBB, c)

    pltpu.make_async_copy(buf, o_hbm.at[pl.ds(0, NBB)], sem.at[WSEM]).wait()
    pltpu.make_async_copy(
        hbuf.at[pl.ds(0, SB)], o_hbm.at[pl.ds(NBB, SB)], sem.at[WSEM]
    ).wait()


@jax.jit
def pallas_standalone__depthwise_separable__vision_kernel(
    x: jax.Array,
    dw: jax.Array,
    pw: jax.Array,
):
    B, Hh, Ww, C = x.shape
    assert dw.shape == (1, 1, C) and pw.shape == (C, C)
    NB = (B * Hh * Ww) // D
    assert NB * D == B * Hh * Ww and NB % SB == 0

    out = pl.pallas_call(
        _kernel,
        in_specs=[pl.BlockSpec(memory_space=pl.ANY)] * 3,
        out_specs=pl.BlockSpec(memory_space=pl.ANY),
        out_shape=jax.ShapeDtypeStruct((NB, D, C), x.dtype),
        scratch_shapes=[
            pltpu.VMEM((NB - SB, D, C), x.dtype),
            pltpu.VMEM((SB + 1, D, C), x.dtype),
            pltpu.VMEM(dw.shape, dw.dtype),
            pltpu.VMEM(pw.shape, pw.dtype),
            pltpu.VMEM(pw.shape, x.dtype),
            pltpu.SMEM((1,), jnp.int32),
            pltpu.SemaphoreType.DMA((3,)),
        ],
        compiler_params=pltpu.CompilerParams(vmem_limit_bytes=114 * 1024 * 1024),
    )(x.reshape(NB, D, C), dw, pw)
    return out.reshape(B, Hh, Ww, C)
```

```python
import jax
import jax.numpy as jnp
import jax.experimental.pallas as pl
import jax.experimental.pallas.tpu as pltpu

D = 2048
SB = 12
TR = 16
G0 = 8
GS = 14
KH = 47
U = 128
TS = 64
X = 8
HR = 2 * X * (U // TS)
NSPLIT = 256
SPIN = 6
PACE_UNROLL = 12
TAIL = 48
S = 6
T = 512
WPAT = (40, 40, 48) * 4
FIRST = 6

PPD = D // TR
UPD = D // U
HI = (KH + 1) * HR
assert PPD == 128 and UPD == 16 and D // T == 4 and SB == 2 * S
assert sum(WPAT) == T and G0 * TR >= U and GS * TR >= U
assert HR == 32 and (D - TAIL - HI) % TR == 0
WSEM = (KH + 1) % 2
HSEM = 2


def _kernel(x_hbm, dw_hbm, pw_hbm, o_hbm, buf, hbuf, dw_v, pw_v, cnt, sem):
    NBB, _, C = buf.shape
    npiece = NBB // SB * PPD
    nunit = NBB // SB * UPD
    nchunk = NBB // S * (D // T)
    nchunk_h = SB // S * (D // T)
    nbulk = npiece + (D - TAIL - HI) // TR
    KD = min(KH, 1 + (npiece - G0) // GS)

    def piece(p, s):
        row = (p & (PPD - 1)) * TR
        if not isinstance(p, int):
            row = pl.multiple_of(row, TR)
        sl = (pl.ds((p >> 7) * SB, SB), pl.ds(row, TR))
        return pltpu.make_async_copy(x_hbm.at[sl], buf.at[sl], sem.at[s])

    def rows_h(row, n, s):
        return pltpu.make_async_copy(
            x_hbm.at[pl.ds(NBB, SB), pl.ds(row, n)],
            hbuf.at[pl.ds(0, SB), pl.ds(row, n)],
            sem.at[s],
        )

    def bulk(lo, hi, s):
        return [
            piece(p, s) if p < npiece else rows_h(HI + (p - npiece) * TR, TR, s)
            for p in range(lo, hi)
        ]

    def group(g):
        return bulk(G0 + (g - 1) * GS, G0 + g * GS, g % 2)

    def rest():
        return bulk(G0 + KH * GS, nbulk, KH % 2)

    def tail():
        return [rows_h(r, 16, HSEM) for r in range(D - TAIL, D, 16)]

    def write_chunk(src, off, c):
        blk = (c >> 3) * SB + (c & 1) * S
        row = ((c >> 1) & 3) * T
        for size in WPAT:
            r = row if isinstance(row, int) else pl.multiple_of(row, 8)
            pltpu.make_async_copy(
                src.at[pl.ds(blk, S), pl.ds(r, size)],
                o_hbm.at[pl.ds(off + blk, S), pl.ds(r, size)],
                sem.at[WSEM],
            ).start()
            row = row + size

    def unit(ref, u):
        row = pl.multiple_of((u & (UPD - 1)) * U, U)
        return ref.at[pl.ds((u >> 4) * SB, SB), pl.ds(row, U)]

    def depthwise(a):
        return (a.astype(jnp.float32) * dw_v[0].astype(jnp.float32)).astype(a.dtype)

    def matmul(a, w):
        return jnp.dot(a, w, preferred_element_type=jnp.float32).astype(buf.dtype)

    cp_dw = pltpu.make_async_copy(dw_hbm, dw_v, sem.at[HSEM])
    cp_pw = pltpu.make_async_copy(pw_hbm, pw_v, sem.at[HSEM])
    cp_dw.start()
    cp_pw.start()
    for c in bulk(0, G0, 0) + group(1):
        c.start(priority=1)
    cnt[0] = 0
    cp_dw.wait()
    cp_pw.wait()
    hbuf[SB, pl.ds(0, C), :] = pw_v[...]

    def paced_read(i, carry):
        r = pl.ds(pl.multiple_of((i & 1) * (HR // 2), HR // 2), HR // 2)
        pltpu.make_async_copy(
            x_hbm.at[NBB + (i >> 1), r], hbuf.at[i >> 1, r], sem.at[HSEM]
        ).start()

        def spin(_, c):
            cnt[0] = cnt[0] + 1
            return c

        return jax.lax.fori_loop(0, SPIN, spin, carry)

    jax.lax.fori_loop(0, 2 * SB, paced_read, 0, unroll=PACE_UNROLL)
    for c in bulk(0, G0, 0):
        c.wait()

    def read_step(k, carry):
        @pl.when((k >= 2) & (k <= KD))
        def _():
            for i in range(GS):
                piece(G0 + (k - 2) * GS + i, (k - 1) & 1).wait()

        for g in range(KD, KH):
            @pl.when(k == g + 1)
            def _():
                for c in group(g):
                    c.wait()

        @pl.when(k + 1 < KD)
        def _():
            for i in range(GS):
                piece(G0 + k * GS + i, (k + 1) & 1).start(priority=1)

        for g in range(KD, KH + 1):
            @pl.when(k + 1 == g)
            def _():
                for c in group(g):
                    c.start(priority=1)

        @pl.when(k == KH)
        def _():
            for c in rest() + tail():
                c.start(priority=1)

        v = unit(buf, k - 1)
        hrows = pl.ds(pl.multiple_of(k * HR, HR), HR)
        hsrc = x_hbm.at[pl.ds(NBB, SB), hrows]
        hdst = hbuf.at[pl.ds(0, SB), hrows]

        def small_read(b, row):
            pltpu.make_async_copy(
                hsrc.at[b, pl.ds(row, X)], hdst.at[b, pl.ds(row, X)], sem.at[HSEM]
            ).start()

        lo, hi = pl.ds(0, NSPLIT), pl.ds(NSPLIT, C - NSPLIT)
        for b in range(SB):
            for s in range(U // TS):
                r = pl.ds(s * TS, TS)
                a = depthwise(v[b, r, :])
                small_read(b, 2 * s * X)
                y_lo = matmul(a, hbuf[SB, pl.ds(0, C), lo])
                small_read(b, (2 * s + 1) * X)
                y_hi = matmul(a, hbuf[SB, pl.ds(0, C), hi])
                v[b, r, lo] = y_lo
                v[b, r, hi] = y_hi
        return carry

    jax.lax.fori_loop(1, KH + 1, read_step, 0)

    for c in group(KH) + rest():
        c.wait()
    for c in range(FIRST):
        write_chunk(buf, 0, c)
    for c in tail():
        c.wait()
    rows_h(0, HI, HSEM).wait()

    def unit_matmul(ref, u):
        v = unit(ref, u)
        for b in range(SB):
            v[b] = matmul(depthwise(v[b]), pw_v[...])

    def buf_step(m, carry):
        unit_matmul(buf, KH + m)

        @pl.when((m & 7) != 7)
        def _():
            write_chunk(buf, 0, FIRST + m - (m >> 3))

        return carry

    nb = nunit - KH
    assert all(FIRST + m - (m >> 3) < (KH + m + 1) // 4 * 2 for m in range(nb))
    jax.lax.fori_loop(0, nb, buf_step, 0)

    def hbuf_step(j, c):
        unit_matmul(hbuf, j)
        ready = c - nchunk < ((j + 1) >> 2) * 2

        @pl.when(c < nchunk)
        def _():
            write_chunk(buf, 0, c)

        @pl.when((c >= nchunk) & ready)
        def _():
            write_chunk(hbuf, NBB, c - nchunk)

        return jnp.where(ready, c + 1, c)

    nxt = FIRST + nb - (nb >> 3)
    jax.lax.fori_loop(0, UPD, hbuf_step, jnp.int32(nxt))
    for j in range(UPD):
        nxt += nxt - nchunk < (j + 1) // 4 * 2
    assert nxt >= nchunk
    for c in range(nxt - nchunk, nchunk_h):
        write_chunk(hbuf, NBB, c)

    pltpu.make_async_copy(buf, o_hbm.at[pl.ds(0, NBB)], sem.at[WSEM]).wait()
    pltpu.make_async_copy(
        hbuf.at[pl.ds(0, SB)], o_hbm.at[pl.ds(NBB, SB)], sem.at[WSEM]
    ).wait()


@jax.jit
def pallas_standalone__depthwise_separable__vision_kernel(
    x: jax.Array,
    dw: jax.Array,
    pw: jax.Array,
):
    B, Hh, Ww, C = x.shape
    assert dw.shape == (1, 1, C) and pw.shape == (C, C) and pw.dtype == x.dtype
    NB = (B * Hh * Ww) // D
    assert NB * D == B * Hh * Ww and NB % SB == 0

    out = pl.pallas_call(
        _kernel,
        in_specs=[pl.BlockSpec(memory_space=pl.ANY)] * 3,
        out_specs=pl.BlockSpec(memory_space=pl.ANY),
        out_shape=jax.ShapeDtypeStruct((NB, D, C), x.dtype),
        scratch_shapes=[
            pltpu.VMEM((NB - SB, D, C), x.dtype),
            pltpu.VMEM((SB + 1, D, C), x.dtype),
            pltpu.VMEM(dw.shape, dw.dtype),
            pltpu.VMEM(pw.shape, pw.dtype),
            pltpu.SMEM((1,), jnp.int32),
            pltpu.SemaphoreType.DMA((3,)),
        ],
        compiler_params=pltpu.CompilerParams(vmem_limit_bytes=114 * 1024 * 1024),
    )(x.reshape(NB, D, C), dw, pw)
    return out.reshape(B, Hh, Ww, C)
```
